```python
import os as _os
_os.environ.setdefault("JAX_PLATFORMS", "cpu")
import jax
import jax.numpy as jnp

def _softmax(x, axis=-1):
    return jax.nn.softmax(x, axis=axis)
def _gelu(x):
    return jax.nn.gelu(x, approximate=True)
def _silu(x):
    return jax.nn.silu(x)
def _sigmoid(x):
    return jax.nn.sigmoid(x)
def _layernorm(x, axis=-1, eps=1e-5):
    m = jnp.mean(x, axis=axis, keepdims=True)
    v = jnp.var(x, axis=axis, keepdims=True)
    return (x - m) / jnp.sqrt(v + eps)
def _scatter_add(tgt, idx, src, axis=0):
    return tgt.at[idx].add(src)
def _segment_sum(src, seg, n):
    return jax.ops.segment_sum(src, seg, n)
class _Rng:
    def __init__(self, key):
        self._k = key
    def _next(self):
        self._k, sub = jax.random.split(self._k)
        return sub
    def normal(self, shape):
        return jax.random.normal(self._next(), shape, dtype=jnp.bfloat16)
    def randint(self, lo, hi, shape):
        return jax.random.randint(self._next(), shape, lo, hi, dtype=jnp.int32)
    def uniform(self, shape, lo=0.0, hi=1.0):
        return jax.random.uniform(self._next(), shape, jnp.bfloat16, lo, hi)
    def permutation(self, n):
        return jax.random.permutation(self._next(), n)


kernel_name = 'sequential_preLN__linear_attn_block__dense_activation_squared_relu__prompt'

def setup_inputs():
    _rng = _Rng(jax.random.key(int.from_bytes(__import__("os").urandom(4), "little")))
    _w = (lambda a: (lambda t: t.astype(jnp.bfloat16) if jnp.issubdtype(t.dtype, jnp.floating) else t)(jnp.asarray(a)))
    def _A_setup():
        B, S, D = 1, 2048, 576
        return {
            "x": _w((lambda *s: _rng.normal(s) * 0.05)(B, S, D)),
            "wqkv": _w((lambda *s: _rng.normal(s) * 0.1)(D, 3 * D)),
            "wo": _w((lambda *s: _rng.normal(s) * 0.05)(D, D)),
        }
    _A_in = _A_setup()

    def _B_setup():
        B, S, D, F = 1, 2048, 576, 4608
        return {
            "x": _w((lambda *s: _rng.normal(s) * 0.05)(B, S, D)),
            "w1": _w((lambda *s: _rng.normal(s) * 0.05)(D, F)),
            "b1": _w((lambda *s: _rng.normal(s) * 0.05)(F)),
            "w2": _w((lambda *s: _rng.normal(s) * 0.05)(F, D)),
            "b2": _w((lambda *s: _rng.normal(s) * 0.05)(D)),
        }
    _B_in = _B_setup()

    return {
        "A_x": _A_in["x"],
        "A_wqkv": _A_in["wqkv"],
        "A_wo": _A_in["wo"],
        "B_x": _B_in["x"],
        "B_w1": _B_in["w1"],
        "B_b1": _B_in["b1"],
        "B_w2": _B_in["w2"],
        "B_b2": _B_in["b2"],
    }

def reference(A_x, A_wqkv, A_wo, B_x, B_w1, B_b1, B_w2, B_b2):
    def _A_ref(x, wqkv, wo):
        B, S, D = x.shape
        H = 32; Dh = D // H
        qkv = (lambda x, *d: x.transpose(*d))((x @ wqkv).reshape(B, S, 3, H, Dh), 2, 0, 3, 1, 4)
        q, k, v = qkv[0], qkv[1], qkv[2]
        phi = lambda t: jnp.where(t > 0, t + 1, jnp.exp(t)) + 1e-6
        pq, pk = phi(q), phi(k)
        kv = jnp.einsum("bhsd,bhse->bhde", pk, v)
        z = jnp.einsum("bhsd->bhd", pk)
        num = jnp.einsum("bhqd,bhde->bhqe", pq, kv)
        den = jnp.einsum("bhqd,bhd->bhq", pq, z)[..., None] + 1e-6
        o = num / den
        return (lambda x, *d: x.transpose(*d))(o, 0, 2, 1, 3).reshape(B, S, D) @ wo

    def _B_ref(x, w1, b1, w2, b2):
        h = jnp.einsum("bsd,df->bsf", x, w1) + b1
        zero = jnp.zeros_like(h)
        r = jnp.where(h > zero, h, zero)
        h = r * r
        out = jnp.einsum("bsf,fd->bsd", h, w2) + b2
        return out

    x = A_x
    h = x + _A_ref(_layernorm(x, axis=-1), A_wqkv, A_wo)
    h2 = h + _B_ref(_layernorm(h, axis=-1), B_w1, B_b1, B_w2, B_b2)
    return h2
```

```python
import jax
import jax.numpy as jnp
from jax import lax
import jax.experimental.pallas as pl
import jax.experimental.pallas.tpu as pltpu

S, D, F = 2048, 576, 4608
H, DH = 32, 18
DP = 640
NT = S // 128
X0 = 384
TN = 256
FC = 1152
OUT_SPLIT = 2
bf16, f32, i32 = jnp.bfloat16, jnp.float32, jnp.int32

BANDS = ((0, 144), (112, 272), (240, 400), (368, 528), (496, 576))
KRANGES = ((0, 256), (0, 384), (128, 512), (256, 576), (384, 576))

SCHED = (
    "w:x0", "ln0", "ln1", "ln2", "w:wk", "wkT",
    "kp0", "kp1", "kp2", "kx0:2:0:5", "kx2:1:0:1", "w:xr", "kx2:1:1:5",
    "ln3", "kp3", "ln4", "kp4", "kx3:1:0:5", "ln5", "kp5", "ln6", "ln7", "ln8", "kp6", "ln9", "kp7",
    "ln10", "kp8", "kx4:4:0:5", "ln11", "kp9", "ln12", "kp10", "ln13", "kp11", "ln14", "kp12",
    "ln15", "kp13", "kx8:4:0:5", "w:wts", "kx12:2:0:5", "wqT", "woT", "bias", "kp14", "kp15",
    "kx14:2:0:5", "z",
    "q0", "w1T0", "q1", "w1T1", "q2", "w1T2", "q3", "w1T3", "q4", "w1T4", "q5", "w1T5",
    "q6", "w1T6", "kv", "q7", "w1T7", "q8", "w1T8", "q9", "q10", "q11", "q12", "mt",
    "q13", "q14", "q15",
)


def _dot(a, b):
    return lax.dot_general(a, b, (((1,), (0,)), ((), ())), preferred_element_type=f32)


def _dot_nt(a, b):
    return lax.dot_general(a, b, (((1,), (1,)), ((), ())), preferred_element_type=f32)


def _b(x):
    return pltpu.bitcast(x, bf16)


def _p(x):
    return pltpu.bitcast(x, i32)


def _phi(t):
    return jnp.where(t > 0, t + 1.0, jnp.exp(t)) + 1e-6


def _head_of(idx):
    return jnp.floor((idx.astype(f32) + 0.5) * (1.0 / DH))


def _ln_stats(xf):
    c = xf[0:1, :]
    d = xf - c
    s1 = jnp.sum(d.reshape(D // 8, 8, 128), axis=0)
    s2 = jnp.sum((d * d).reshape(D // 8, 8, 128), axis=0)
    m = jnp.sum(s1, axis=0, keepdims=True) * (1.0 / D)
    var = jnp.maximum(jnp.sum(s2, axis=0, keepdims=True) * (1.0 / D) - m * m, 0.0)
    return m + c, lax.rsqrt(var + 1e-5)


def _kernel(xT_hbm, wqkv_hbm, wo_hbm, w1_hbm, b1_hbm, w2T_hbm, b2_hbm, out_hbm,
            xT_v, wqkv_v, wo_v, w1_v, w2T_v, b1_v, b2_v,
            wqkT_v, woT_v, w1T_v, xnT_v, pk_v, KX_v, Z_v, kv_v, MT_v, PQ_v, hnT_v, H_v, b2c_v, out_v,
            st_v, sems):
    n_blk = S // TN
    tpb = TN // 128
    ots = TN // OUT_SPLIT
    copies = []

    def copy(src, dst):
        copies.append(pltpu.make_async_copy(src, dst, sems.at[len(copies)]))
        return copies[-1]

    cp_x0 = copy(xT_hbm.at[:, pl.ds(0, X0)], xT_v.at[:, pl.ds(0, X0)])
    cp_wk = copy(wqkv_hbm.at[:, pl.ds(512, 640)], wqkv_v.at[:, pl.ds(512, 640)])
    cp_xr = copy(xT_hbm.at[:, pl.ds(X0, S - X0)], xT_v.at[:, pl.ds(X0, S - X0)])
    cp_wq = copy(wqkv_hbm.at[:, pl.ds(0, 512)], wqkv_v.at[:, pl.ds(0, 512)])
    cp_wv = copy(wqkv_hbm.at[:, pl.ds(1152, 576)], wqkv_v.at[:, pl.ds(1152, 576)])
    cp_wo = copy(wo_hbm, wo_v)
    cp_b1 = copy(b1_hbm, b1_v)
    cp_b2 = copy(b2_hbm, b2_v)
    cp_w1 = copy(w1_hbm, w1_v.at[pl.ds(0, D), :])
    cp_w2 = copy(w2T_hbm, w2T_v)
    osem = len(copies)
    waits = dict(x0=[cp_x0], wk=[cp_wk], xr=[cp_xr], wts=[cp_wq, cp_wv, cp_wo, cp_b1, cp_b2, cp_w1])
    for c in copies:
        c.start()

    def out_slice(b, j):
        off = b * TN + j * ots
        return pl.ds(off if isinstance(off, int) else pl.multiple_of(off, ots), ots)

    def cp_out(b, j):
        return pltpu.make_async_copy(out_v.at[:, out_slice(b, j)], out_hbm.at[:, out_slice(b, j)],
                                     sems.at[osem + b * OUT_SPLIT + j])

    xnT_v[D // 2:DP // 2, :] = _p(jnp.ones((DP - D, S), bf16))
    hnT_v[D // 2:DP // 2, :] = _p(jnp.ones((DP - D, TN), bf16))
    kv_v[...] = jnp.zeros(kv_v.shape, i32)

    def tile(t):
        return slice(t * 128, (t + 1) * 128)

    def ln1(t):
        sl = tile(t)
        mean, rstd = _ln_stats(xT_v[:, sl].astype(f32))
        st_v[0:1, :] = rstd
        xn = (xT_v[:, sl].astype(f32) - mean) * rstd
        xnT_v[0:D // 2, sl] = _p(xn.astype(bf16))

    def kproj(t):
        sl = tile(t)
        k = _dot(_b(wqkT_v[D // 2:D, :]), _b(xnT_v[0:D // 2, sl]))
        pk_v[:, sl] = _p(_phi(k).astype(bf16))

    def kxf(t0, n, j0, j1):
        sl = slice(t0 * 128, (t0 + n) * 128)
        js = slice(j0 * 128, j1 * 128)
        part = _dot_nt(_b(pk_v[:, sl]), _b(xnT_v[j0 * 64:j1 * 64, sl]))
        if t0 == 0:
            KX_v[:, js] = part
        else:
            KX_v[:, js] = KX_v[:, js] + part

    def bias():
        b2r = jnp.broadcast_to(b2_v[...].astype(f32).reshape(1, D), (128, D))
        b2c_v[...] = b2r.T
        b1r = jnp.broadcast_to(b1_v[...].astype(f32).reshape(1, F), (DP - D, F))
        row = lax.broadcasted_iota(i32, (DP - D, F), 0)
        w1_v[D:DP, :] = jnp.where(row == 0, b1r, 0.0).astype(bf16)

    def zf():
        t4 = KX_v[:, 512:640]
        lane = lax.broadcasted_iota(i32, (D, 128), 1)
        Z_v[...] = jnp.where(lane >= 64, t4, pltpu.roll(t4, 64, 1))

    def kvf():
        for kt, (r0, r1) in enumerate(BANDS):
            w = 128 if kt < 4 else 64
            c0 = 1152 + 128 * kt
            blk = _dot(KX_v[r0:r1, 0:D].astype(bf16), wqkv_v[:, c0:c0 + w])
            rh = _head_of(lax.broadcasted_iota(i32, (r1 - r0, w), 0) + r0)
            ch = _head_of(lax.broadcasted_iota(i32, (r1 - r0, w), 1) + 128 * kt)
            kv_v[r0 // 2:r1 // 2, 128 * kt:128 * kt + w] = _p(jnp.where(rh == ch, blk, 0.0).astype(bf16))

    def mtf():
        for j, (k0, k1) in enumerate(KRANGES[:4]):
            mt = _dot_nt(_b(woT_v[:, k0:k1]), _b(kv_v[64 * j:64 * j + 64, k0:k1]))
            MT_v[:, 128 * j:128 * j + 128] = _p(mt.astype(bf16))
        mt = _dot_nt(_b(woT_v[:, 384:512]), _b(kv_v[256:288, 384:512]))
        for qd in range(4):
            r0, r1 = 144 * qd, 144 * (qd + 1)
            m2 = _dot_nt(_b(woT_v[r0 // 2:r1 // 2, 512:576]), _b(kv_v[256:288, 512:576]))
            MT_v[r0 // 2:r1 // 2, 512:576] = _p((mt[r0:r1, :] + m2).astype(bf16))

    def qproj(t):
        q = _dot(_b(wqkT_v[0:D // 2, :]), _b(xnT_v[0:D // 2, tile(t)]))
        sub = lax.broadcasted_iota(i32, (8, 128), 0)
        outs = []
        for g in range(D // 72):
            p = [_phi(q[72 * g + 8 * j:72 * g + 8 * j + 8, :]) for j in range(9)]
            v = [p[j] * Z_v[72 * g + 8 * j:72 * g + 8 * j + 8, :] for j in range(9)]
            sa = v[0] + v[1] + jnp.where(sub < 2, v[2], 0.0)
            sb = jnp.where(sub >= 2, v[2], 0.0) + v[3] + jnp.where(sub < 4, v[4], 0.0)
            sc = jnp.where(sub >= 4, v[4], 0.0) + v[5] + jnp.where(sub < 6, v[6], 0.0)
            sd = jnp.where(sub >= 6, v[6], 0.0) + v[7] + v[8]
            ra, rb, rc, rd = [1.0 / (jnp.sum(s, axis=0, keepdims=True) + 1e-6) for s in (sa, sb, sc, sd)]
            outs += [p[0] * ra, p[1] * ra, p[2] * jnp.where(sub < 2, ra, rb), p[3] * rb,
                     p[4] * jnp.where(sub < 4, rb, rc), p[5] * rc, p[6] * jnp.where(sub < 6, rc, rd),
                     p[7] * rd, p[8] * rd]
        PQ_v[:, tile(t)] = _p(jnp.concatenate(outs, axis=0).astype(bf16))

    for task in SCHED:
        if task.startswith("w:"):
            for c in waits[task[2:]]:
                c.wait()
        elif task == "wkT":
            wqkT_v[256:D, :] = _p(wqkv_v[:, 512:1152].T)
        elif task == "wqT":
            wqkT_v[0:256, :] = _p(wqkv_v[:, 0:512].T)
        elif task == "woT":
            woT_v[...] = _p(wo_v[...].T)
        elif task == "bias":
            bias()
        elif task == "z":
            zf()
        elif task == "kv":
            kvf()
        elif task == "mt":
            mtf()
        elif task.startswith("w1T"):
            c = int(task[3:])
            w1T_v[c * 256:(c + 1) * 256, :] = _p(w1_v[:, c * 512:(c + 1) * 512].T)
        elif task.startswith("ln"):
            ln1(int(task[2:]))
        elif task.startswith("kp"):
            kproj(int(task[2:]))
        elif task.startswith("kx"):
            kxf(*[int(v) for v in task[2:].split(":")])
        elif task.startswith("q"):
            qproj(int(task[1:]))
        else:
            raise ValueError(task)

    cp_w2.wait()

    def block(b, carry):
        bs = pl.ds(pl.multiple_of(b * TN, TN), TN)
        pqb = _b(PQ_v[:, bs])
        attn = jnp.concatenate([_dot(_b(MT_v[i * D // 4:(i + 1) * D // 4, :]), pqb) for i in range(2)], axis=0)
        xb = xT_v[:, bs]
        for lt in range(tpb):
            sl = tile(lt)
            h = xb[:, sl].astype(f32) + attn[:, sl]
            H_v[:, sl] = h
            mean, rstd = _ln_stats(h)
            st_v[0:1, :] = rstd
            hn = (H_v[:, sl] - mean) * rstd
            hnT_v[0:D // 2, sl] = _p(hn.astype(bf16))
        acts = []
        for c in range(F // FC):
            hid = _dot(_b(w1T_v[c * FC // 2:(c + 1) * FC // 2, :]), _b(hnT_v[...]))
            r = jnp.maximum(hid, 0.0)
            acts.append((r * r).astype(bf16))
        for j in range(OUT_SPLIT):
            osl = slice(j * ots, (j + 1) * ots)
            o = H_v[:, osl] + jnp.concatenate([b2c_v[...]] * (ots // 128), axis=1)
            for c in range(F // FC):
                o = o + _dot(w2T_v[:, c * FC:(c + 1) * FC], acts[c][:, osl])
            out_v[:, out_slice(b, j)] = o.astype(bf16)
            cp_out(b, j).start()
        return carry

    lax.fori_loop(0, n_blk, block, 0)
    for b in range(n_blk):
        for j in range(OUT_SPLIT):
            cp_out(b, j).wait()


@jax.jit
def pallas_sequential_preLN__linear_attn_block__dense_activation_squared_relu__prompt_kernel(
    A_x: jax.Array,
    A_wqkv: jax.Array,
    A_wo: jax.Array,
    B_x: jax.Array,
    B_w1: jax.Array,
    B_b1: jax.Array,
    B_w2: jax.Array,
    B_b2: jax.Array,
):
    del B_x
    any_spec = pl.BlockSpec(memory_space=pl.ANY)
    vm = pltpu.VMEM
    out_t = pl.pallas_call(
        _kernel,
        out_shape=jax.ShapeDtypeStruct((D, S), bf16),
        in_specs=[any_spec] * 7,
        out_specs=any_spec,
        scratch_shapes=[
            vm((D, S), bf16), vm((D, 3 * D), bf16), vm((D, D), bf16), vm((DP, F), bf16), vm((D, F), bf16),
            vm((F,), bf16), vm((D,), bf16),
            vm((D, D), i32), vm((D // 2, D), i32), vm((F // 2, DP), i32), vm((DP // 2, S), i32),
            vm((D // 2, S), i32), vm((D, DP), f32), vm((D, 128), f32), vm((D // 2, D), i32),
            vm((D // 2, D), i32), vm((D // 2, S), i32), vm((DP // 2, TN), i32), vm((D, TN), f32),
            vm((D, 128), f32), vm((D, S), bf16), vm((8, 128), f32),
            pltpu.SemaphoreType.DMA((10 + (S // TN) * OUT_SPLIT,)),
        ],
        compiler_params=pltpu.CompilerParams(vmem_limit_bytes=100 * 1024 * 1024),
    )(A_x.reshape(S, D).T, A_wqkv, A_wo, B_w1, B_b1, B_w2.T, B_b2)
    return out_t.T.reshape(1, S, D)
```
